```python
import jax
import jax.numpy as jnp

def _softmax(x, axis=-1):
    return jax.nn.softmax(x, axis=axis)
def _gelu(x):
    return jax.nn.gelu(x, approximate=True)
def _silu(x):
    return jax.nn.silu(x)
def _sigmoid(x):
    return jax.nn.sigmoid(x)
def _layernorm(x, axis=-1, eps=1e-5):
    m = jnp.mean(x, axis=axis, keepdims=True)
    v = jnp.var(x, axis=axis, keepdims=True)
    return (x - m) / jnp.sqrt(v + eps)
def _scatter_add(tgt, idx, src, axis=0):
    return tgt.at[idx].add(src)
def _segment_sum(src, seg, n):
    return jax.ops.segment_sum(src, seg, n)
class _Rng:
    def __init__(self, key):
        self._k = key
    def _next(self):
        self._k, sub = jax.random.split(self._k)
        return sub
    def normal(self, shape):
        return jax.random.normal(self._next(), shape, dtype=jnp.bfloat16)
    def randint(self, lo, hi, shape):
        return jax.random.randint(self._next(), shape, lo, hi, dtype=jnp.int32)
    def uniform(self, shape, lo=0.0, hi=1.0):
        return jax.random.uniform(self._next(), shape, jnp.bfloat16, lo, hi)
    def permutation(self, n):
        return jax.random.permutation(self._next(), n)


kernel_name = 'parallel_sum__sliding_block_cached__moe_arch_mod__decode'

def setup_inputs():
    _rng = _Rng(jax.random.key(int.from_bytes(__import__("os").urandom(4), "little")))
    _w = (lambda a: (lambda t: t.astype(jnp.bfloat16) if jnp.issubdtype(t.dtype, jnp.floating) else t)(jnp.asarray(a)))
    def _A_setup():
        B, Sq, D = 1, 1, 512
        Hq, Hkv, Sk, Dh = 32, 8, 65536, 128
        assert Hq % Hkv == 0, (Hq, Hkv)
        return {
            "x": _w((lambda *s: _rng.normal(s) * 0.05)(B, Sq, D)),
            "k_cache": _w((lambda *s: _rng.normal(s) * 0.05)(B, Hkv, Sk, Dh)),
            "v_cache": _w((lambda *s: _rng.normal(s) * 0.05)(B, Hkv, Sk, Dh)),
            "wq": _w((lambda *s: _rng.normal(s) * 0.05)(D, Hq * Dh) * (D ** -0.5)),
            "wo": _w((lambda *s: _rng.normal(s) * 0.05)(Hq * Dh, D) * ((Hq * Dh) ** -0.5)),
        }
    _A_in = _A_setup()

    def _B_setup():
        B, S, D, F, C = 1, 1, 512, 1792, 1
        return {
            "x": _w((lambda *s: _rng.normal(s) * 0.05)(B, S, D)),
            "w_r": _w((lambda *s: _rng.normal(s) * 0.05)(D)),
            "w_gate": _w((lambda *s: _rng.normal(s) * 0.05)(D, F)),
            "w_up": _w((lambda *s: _rng.normal(s) * 0.05)(D, F)),
            "w_down": _w((lambda *s: _rng.normal(s) * 0.05)(F, D)),
        }
    _B_in = _B_setup()

    return {
        "A_x": _A_in["x"],
        "A_k_cache": _A_in["k_cache"],
        "A_v_cache": _A_in["v_cache"],
        "A_wq": _A_in["wq"],
        "A_wo": _A_in["wo"],
        "B_x": _B_in["x"],
        "B_w_r": _B_in["w_r"],
        "B_w_gate": _B_in["w_gate"],
        "B_w_up": _B_in["w_up"],
        "B_w_down": _B_in["w_down"],
    }

def reference(A_x, A_k_cache, A_v_cache, A_wq, A_wo, B_x, B_w_r, B_w_gate, B_w_up, B_w_down):
    def _A_ref(x, k_cache, v_cache, wq, wo):
        B, Sq, D = x.shape
        Hq, Dh = 32, 128
        Hkv, Sk = k_cache.shape[1], k_cache.shape[2]
        W = min(4096, max(256, Sk // 4))
        rep = Hq // Hkv
        q = (lambda x, *d: x.transpose(*d))((x @ wq).reshape(B, Sq, Hq, Dh), 0, 2, 1, 3)
        k = jnp.repeat(k_cache[:, :, Sk - W:, :], rep, axis=1)
        v = jnp.repeat(v_cache[:, :, Sk - W:, :], rep, axis=1)
        scores = jnp.einsum("bhqd,bhkd->bhqk", q, k) * (Dh ** -0.5)
        p = _softmax(scores, axis=-1)
        o = jnp.einsum("bhqk,bhkd->bhqd", p, v)
        return (lambda x, *d: x.transpose(*d))(o, 0, 2, 1, 3).reshape(B, Sq, Hq * Dh) @ wo

    def _B_ref(x, w_r, w_gate, w_up, w_down):
        B, S, D = x.shape
        C = 1
        r = x @ w_r
        idx = jnp.argsort(-r, axis=-1)[:, :C]
        idx_e = jnp.repeat(idx.reshape(B, C, 1), D, axis=2)
        x_sel = jnp.take_along_axis(x, idx_e, axis=1)
        g = _silu(x_sel @ w_gate)
        u = x_sel @ w_up
        y = (g * u) @ w_down
        r_sel = _sigmoid(jnp.take_along_axis(r, idx, axis=1))
        y = y * r_sel.reshape(B, C, 1)
        b_off = (jnp.arange(B) * S).reshape(B, 1)
        flat_idx = (idx + b_off).reshape(B * C)
        zero = (x * 0.0).reshape(B * S, D)
        upd = _scatter_add(zero, flat_idx, y.reshape(B * C, D), axis=0)
        return x + upd.reshape(B, S, D)

    x = A_x
    xn = _layernorm(x, axis=-1)
    return x + _A_ref(xn, A_k_cache, A_v_cache, A_wq, A_wo) + _B_ref(xn, B_w_r, B_w_gate, B_w_up, B_w_down)
```

```python
import functools
import jax
import jax.numpy as jnp
from jax import lax
import jax.experimental.pallas as pl
import jax.experimental.pallas.tpu as pltpu

D = 512; HQ = 32; HKV = 8; DH = 128; F = 1792; W = 4096; REP = HQ // HKV

def _kernel(x_ref, wr_ref, k_hbm, v_hbm, wq_hbm, wo_hbm, wg_hbm, wu_hbm, wd_hbm, o_ref,
            kbuf, vbuf, wqbuf, wobuf, wgbuf, wubuf, wdbuf):
    sk = k_hbm.shape[2]
    f32 = jnp.float32; bf16 = jnp.bfloat16

    def body(sems):
        copies = {}
        idx = [0]
        def add(name, src, dst):
            copies[name] = pltpu.make_async_copy(src, dst, sems.at[idx[0]]); idx[0] += 1
        for h in range(HKV):
            add(("q", h), wq_hbm.at[:, pl.ds(h * 512, 512)], wqbuf.at[:, pl.ds(h * 512, 512)])
        for h in range(HKV):
            add(("k", h), k_hbm.at[0, h, pl.ds(sk - W, W), :], kbuf.at[h])
            add(("v", h), v_hbm.at[0, h, pl.ds(sk - W, W), :], vbuf.at[h])
            add(("o", h), wo_hbm.at[pl.ds(h * 512, 512), :], wobuf.at[pl.ds(h * 512, 512), :])
        add("g", wg_hbm, wgbuf)
        add("u", wu_hbm, wubuf)
        for c in range(7):
            add(("d", c), wd_hbm.at[pl.ds(c * 256, 256), :], wdbuf.at[pl.ds(c * 256, 256), :])
        for c in copies.values(): c.start()
        def wait(name):
            copies[name].wait()

        x = x_ref[0].astype(f32)
        m = jnp.mean(x, axis=-1, keepdims=True)
        xc = x - m
        var = jnp.mean(xc * xc, axis=-1, keepdims=True)
        xn = xc / jnp.sqrt(var + 1e-5)
        xn_b = xn.astype(bf16)
        xn8 = jnp.broadcast_to(xn_b.astype(f32), (8, D)).astype(bf16)
        r = jnp.sum(xn_b.astype(f32) * wr_ref[...].astype(f32).reshape(1, D), axis=-1, keepdims=True)
        gate = jax.nn.sigmoid(r)

        row = lax.broadcasted_iota(jnp.int32, (8, DH), 0)
        acc = jnp.zeros((8, D), f32)
        qs = []
        for h in range(HKV):
            wait(("q", h))
            qf = jnp.dot(xn8, wqbuf[:, h * 512:(h + 1) * 512], preferred_element_type=f32)
            qh = jnp.zeros((8, DH), f32)
            for r_ in range(REP):
                qh = jnp.where(row == r_, qf[:, r_ * DH:(r_ + 1) * DH], qh)
            qs.append(qh.astype(bf16))
        for h in range(HKV):
            wait(("k", h))
            s = lax.dot_general(qs[h], kbuf[h], (((1,), (1,)), ((), ())), preferred_element_type=f32) * (DH ** -0.5)
            mx = jnp.max(s, axis=-1, keepdims=True)
            p = jnp.exp(s - mx)
            l = jnp.sum(p, axis=-1, keepdims=True)
            wait(("v", h))
            o = jnp.dot(p.astype(bf16), vbuf[h], preferred_element_type=f32) / l
            ob = jnp.concatenate([jnp.where(row == r_, o, 0.0) for r_ in range(REP)], axis=1).astype(bf16)
            wait(("o", h))
            acc = acc + jnp.dot(ob, wobuf[h * 512:(h + 1) * 512, :], preferred_element_type=f32)
        attn = jnp.sum(acc, axis=0, keepdims=True)
        wait("g"); wait("u")
        g = jnp.dot(xn8, wgbuf[...], preferred_element_type=f32)
        u = jnp.dot(xn8, wubuf[...], preferred_element_type=f32)
        hmid = (jax.nn.silu(g) * u).astype(bf16)
        y = jnp.zeros((8, D), f32)
        for c in range(7):
            wait(("d", c))
            y = y + jnp.dot(hmid[:, c * 256:(c + 1) * 256], wdbuf[c * 256:(c + 1) * 256, :], preferred_element_type=f32)
        out = x + attn + xn_b.astype(f32) + y[0:1, :] * gate
        o_ref[0] = out.astype(o_ref.dtype)

    pl.run_scoped(body, pltpu.SemaphoreType.DMA((64,)))


@jax.jit
def pallas_parallel_sum__sliding_block_cached__moe_arch_mod__decode_kernel(
    A_x, A_k_cache, A_v_cache, A_wq, A_wo, B_x, B_w_r, B_w_gate, B_w_up, B_w_down):
    bf = jnp.bfloat16
    vm = pl.BlockSpec(memory_space=pltpu.VMEM)
    hb = pl.BlockSpec(memory_space=pl.ANY)
    return pl.pallas_call(
        _kernel,
        out_shape=jax.ShapeDtypeStruct((1, 1, D), bf),
        in_specs=[vm, vm] + [hb] * 7,
        out_specs=vm,
        scratch_shapes=[
            pltpu.VMEM((HKV, W, DH), bf), pltpu.VMEM((HKV, W, DH), bf),
            pltpu.VMEM((D, HQ * DH), bf), pltpu.VMEM((HQ * DH, D), bf),
            pltpu.VMEM((D, F), bf), pltpu.VMEM((D, F), bf), pltpu.VMEM((F, D), bf),
        ],
        compiler_params=pltpu.CompilerParams(vmem_limit_bytes=64 * 1024 * 1024),
    )(A_x, B_w_r, A_k_cache, A_v_cache, A_wq, A_wo, B_w_gate, B_w_up, B_w_down)
```

```python
import functools
import jax
import jax.numpy as jnp
from jax import lax
import jax.experimental.pallas as pl
import jax.experimental.pallas.tpu as pltpu

D = 512; HQ = 32; HKV = 8; DH = 128; F = 1792; W = 4096; REP = HQ // HKV
NOCOMP = False
MAXOUT = 96
KVB = 256


def _kernel(x_hbm, wr_hbm, k_hbm, v_hbm, wq_hbm, wo_hbm, wg_hbm, wu_hbm, wd_hbm, o_ref,
            xbuf, wrbuf, kbuf, vbuf, wqbuf, wobuf, wgbuf, wubuf, wdbuf, s_buf):
    sk = k_hbm.shape[2]
    f32 = jnp.float32; bf16 = jnp.bfloat16

    def body(sems):
        st = {}
        groups = []

        def grp(descs, wait_refs, compute):
            groups.append((descs, wait_refs, compute))

        def wdescs(hbm, buf, g0, g1, r0, r1, group, rows, cols):
            C = hbm.shape[2]
            out = []
            for r in range(r0, r1, rows):
                for c in range(0, C, cols):
                    for g in range(g0, g1, group):
                        sl = (pl.ds(g, group), pl.ds(r, rows), pl.ds(c, cols))
                        out.append((hbm.at[sl], buf.at[sl]))
            return out

        row = lax.broadcasted_iota(jnp.int32, (8, DH), 0)

        def c_x():
            x = xbuf[0].astype(f32)
            m = jnp.mean(x, axis=-1, keepdims=True)
            xc = x - m
            var = jnp.mean(xc * xc, axis=-1, keepdims=True)
            xn = (xc / jnp.sqrt(var + 1e-5)).astype(bf16).astype(f32)
            st["x"] = x; st["xn"] = xn
            st["xn8"] = jnp.broadcast_to(xn, (8, D)).astype(bf16)
            r = jnp.sum(xn * wrbuf[...].astype(f32).reshape(1, D), axis=-1, keepdims=True)
            st["gate"] = jax.nn.sigmoid(r)
        grp([(x_hbm, xbuf), (wr_hbm, wrbuf)], [xbuf, wrbuf], c_x)

        def c_q():
            wq = wqbuf[...].reshape(D, HQ * DH)
            qf = jnp.dot(st["xn8"], wq, preferred_element_type=f32)
            qs = []
            for h in range(HKV):
                qh = jnp.zeros((8, DH), f32)
                for r_ in range(REP):
                    c0 = (h * REP + r_) * DH
                    qh = jnp.where(row == r_, qf[:, c0:c0 + DH], qh)
                qs.append(qh.astype(bf16))
            st["q"] = qs
            st["m"] = [jnp.full((8, DH), -jnp.inf, f32) for _ in range(HKV)]
        for r in range(0, 64, 8):
            grp(wdescs(wq_hbm, wqbuf, 0, 8, r, r + 8, 2, 8, 1024), [wqbuf.at[:, pl.ds(r, 8), :]],
                c_q if r == 56 else None)

        def kvdescs(hbm, buf, j0):
            out = []
            for j in range(j0, j0 + KVB, 64):
                for g in range(0, 8, 2):
                    out.append((hbm.at[0, pl.ds(g, 2), pl.ds(sk - W + j, 64), :], buf.at[pl.ds(g, 2), pl.ds(j, 64), :]))
            return out

        def c_k(j0, last):
            def f():
                for h in range(HKV):
                    s = lax.dot_general(st["q"][h], kbuf[h, j0:j0 + KVB, :], (((1,), (1,)), ((), ())),
                                        preferred_element_type=f32) * (DH ** -0.5)
                    s_buf[h, :, j0:j0 + KVB] = s
                    m = st["m"][h]
                    for c in range(KVB // DH):
                        m = jnp.maximum(m, s[:, c * DH:(c + 1) * DH])
                    st["m"][h] = m
                if last:
                    st["mx"] = [jnp.max(st["m"][h], axis=-1, keepdims=True) for h in range(HKV)]
                    st["l"] = [jnp.zeros((8, DH), f32) for _ in range(HKV)]
                    st["o"] = [jnp.zeros((8, DH), f32) for _ in range(HKV)]
            return f
        for j0 in range(0, W, KVB):
            grp(kvdescs(k_hbm, kbuf, j0), [kbuf.at[:, pl.ds(j0, KVB), :]], c_k(j0, j0 + KVB == W))

        def c_v(j0, last):
            def f():
                for h in range(HKV):
                    p = jnp.exp(s_buf[h, :, j0:j0 + KVB] - st["mx"][h])
                    l = st["l"][h]
                    for c in range(KVB // DH):
                        l = l + p[:, c * DH:(c + 1) * DH]
                    st["l"][h] = l
                    st["o"][h] = st["o"][h] + jnp.dot(p.astype(bf16), vbuf[h, j0:j0 + KVB, :], preferred_element_type=f32)
                if last:
                    st["on"] = [st["o"][h] / jnp.sum(st["l"][h], axis=-1, keepdims=True) for h in range(HKV)]
                    st["acc"] = jnp.zeros((8, D), f32)
            return f
        for j0 in range(0, W, KVB):
            grp(kvdescs(v_hbm, vbuf, j0), [vbuf.at[:, pl.ds(j0, KVB), :]], c_v(j0, j0 + KVB == W))

        def c_o(r_):
            def f():
                acc = st["acc"]
                for h in range(HKV):
                    ob = jnp.where(row == r_, st["on"][h], 0.0).astype(bf16)
                    acc = acc + jnp.dot(ob, wobuf[h, r_ * DH:(r_ + 1) * DH, :], preferred_element_type=f32)
                st["acc"] = acc
            return f
        for r in range(0, 512, 64):
            grp(wdescs(wo_hbm, wobuf, 0, 8, r, r + 64, 2, 16, 512), [wobuf.at[:, pl.ds(r, 64), :]],
                c_o(r // DH) if (r + 64) % DH == 0 else None)

        def c_g():
            st["g"] = jnp.dot(st["xn8"], wgbuf[...].reshape(D, F), preferred_element_type=f32)
        def c_u():
            u = jnp.dot(st["xn8"], wubuf[...].reshape(D, F), preferred_element_type=f32)
            st["h"] = (jax.nn.silu(st["g"]) * u).astype(bf16)
            st["y"] = jnp.zeros((8, D), f32)
        for hbm, buf, cf in ((wg_hbm, wgbuf, c_g), (wu_hbm, wubuf, c_u)):
            for r in range(0, 64, 16):
                grp(wdescs(hbm, buf, 0, 8, r, r + 16, 2, 8, 896), [buf.at[:, pl.ds(r, 16), :]],
                    cf if r == 48 else None)

        def c_d(b0, b1):
            def f():
                y = st["y"]
                y = y + jnp.dot(st["h"][:, b0 * DH:b1 * DH], wdbuf[b0:b1].reshape((b1 - b0) * DH, D),
                                preferred_element_type=f32)
                st["y"] = y
            return f
        for b0, b1 in ((0, 4), (4, 8), (8, 12), (12, 14)):
            grp(wdescs(wd_hbm, wdbuf, b0, b1, 0, 128, 2, 16, 512), [wdbuf.at[pl.ds(b0, b1 - b0)]], c_d(b0, b1))

        n = len(groups)
        cnt = [0]
        def issue(i):
            for s, d in groups[i][0]:
                pltpu.make_async_copy(s, d, sems.at[i]).start(priority=cnt[0] % 2)
                cnt[0] += 1
        issued = 0
        def fill(done):
            nonlocal issued
            while issued < n and sum(len(groups[j][0]) for j in range(done, issued + 1)) <= MAXOUT:
                issue(issued); issued += 1
        fill(0)
        for i in range(n):
            assert issued > i
            for wr in groups[i][1]:
                pltpu.make_async_copy(wr, wr, sems.at[i]).wait()
            fill(i + 1)
            if groups[i][2] is not None and not (NOCOMP and i > 0):
                groups[i][2]()
        if NOCOMP:
            o_ref[0] = st["x"].astype(o_ref.dtype)
        else:
            attn = jnp.sum(st["acc"], axis=0, keepdims=True)
            out = st["x"] + attn + st["xn"] + st["y"][0:1, :] * st["gate"]
            o_ref[0] = out.astype(o_ref.dtype)

    pl.run_scoped(body, pltpu.SemaphoreType.DMA((80,)))


@jax.jit
def pallas_parallel_sum__sliding_block_cached__moe_arch_mod__decode_kernel(
    A_x, A_k_cache, A_v_cache, A_wq, A_wo, B_x, B_w_r, B_w_gate, B_w_up, B_w_down):
    bf = jnp.bfloat16
    vm = pl.BlockSpec(memory_space=pltpu.VMEM)
    hb = pl.BlockSpec(memory_space=pl.ANY)
    return pl.pallas_call(
        _kernel,
        out_shape=jax.ShapeDtypeStruct((1, 1, D), bf),
        in_specs=[hb] * 9,
        out_specs=vm,
        scratch_shapes=[
            pltpu.VMEM((1, 1, D), bf), pltpu.VMEM((D,), bf),
            pltpu.VMEM((HKV, W, DH), bf), pltpu.VMEM((HKV, W, DH), bf),
            pltpu.VMEM((8, D // 8, HQ * DH), bf), pltpu.VMEM((8, 512, D), bf),
            pltpu.VMEM((8, D // 8, F), bf), pltpu.VMEM((8, D // 8, F), bf), pltpu.VMEM((14, 128, D), bf),
            pltpu.VMEM((HKV, 8, W), jnp.float32),
        ],
        compiler_params=pltpu.CompilerParams(vmem_limit_bytes=64 * 1024 * 1024),
    )(A_x, B_w_r, A_k_cache, A_v_cache, A_wq.reshape(8, D // 8, HQ * DH), A_wo.reshape(8, 512, D),
      B_w_gate.reshape(8, D // 8, F), B_w_up.reshape(8, D // 8, F), B_w_down.reshape(14, 128, D))
```

```python
import jax
import jax.numpy as jnp
from jax import lax
import jax.experimental.pallas as pl
import jax.experimental.pallas.tpu as pltpu

HQ = 32
DH = 128
LN_EPS = 1e-5

NSTREAM = 8
KV_BLOCK = 256
KV_ROWS = 64
LOOKAHEAD = 96
LOW_START = 32
TAIL_BLOCKS = 2
TAIL_ROWS = 32


def _kernel(x_hbm, wr_hbm, k_hbm, v_hbm, wq_hbm, wo_hbm, wg_hbm, wu_hbm, wd_hbm, o_ref,
            xbuf, wrbuf, kbuf, vbuf, wqbuf, wobuf, wgbuf, wubuf, wdbuf, s_buf):
    f32, bf16 = jnp.float32, jnp.bfloat16
    d_model = xbuf.shape[-1]
    hkv, win, _ = kbuf.shape
    sk = k_hbm.shape[2]
    rep = HQ // hkv
    d_ff = wgbuf.shape[-1]
    n_dblk = wdbuf.shape[0]
    n_mxu_dblk = n_dblk - TAIL_BLOCKS

    st = {}
    row = lax.broadcasted_iota(jnp.int32, (8, DH), 0)
    row_d = lax.broadcasted_iota(jnp.int32, (8, d_model), 0)

    def band_copies(hbm, buf, g0, g1, r0, r1, rows, cols):
        out = []
        for r in range(r0, r1, rows):
            for c in range(0, hbm.shape[2], cols):
                for g in range(g0, g1, 2):
                    sl = (pl.ds(g, 2), pl.ds(r, rows), pl.ds(c, cols))
                    out.append((hbm.at[sl], buf.at[sl]))
        return out

    def kv_copies(hbm, buf, j0):
        out = []
        for j in range(j0, j0 + KV_BLOCK, KV_ROWS):
            for g in range(0, hkv, 2):
                out.append((hbm.at[0, pl.ds(g, 2), pl.ds(sk - win + j, KV_ROWS), :],
                            buf.at[pl.ds(g, 2), pl.ds(j, KV_ROWS), :]))
        return out

    def step_x():
        x = xbuf[0].astype(f32)
        xc = x - jnp.mean(x, axis=-1, keepdims=True)
        var = jnp.mean(xc * xc, axis=-1, keepdims=True)
        xn = (xc / jnp.sqrt(var + LN_EPS)).astype(bf16).astype(f32)
        st["xn8"] = jnp.broadcast_to(xn, (8, d_model)).astype(bf16)
        r = jnp.sum(xn * wrbuf[...].astype(f32).reshape(1, d_model), axis=-1, keepdims=True)
        st["gate"] = jax.nn.sigmoid(r)
        st["acc"] = jnp.where(row_d == 0, jnp.broadcast_to(x + xn, (8, d_model)), 0.0)

    def step_q():
        qf = jnp.dot(st["xn8"], wqbuf[...].reshape(d_model, HQ * DH),
                     preferred_element_type=f32)
        st["q"] = []
        for h in range(hkv):
            qh = jnp.zeros((8, DH), f32)
            for r in range(rep):
                c0 = (h * rep + r) * DH
                qh = jnp.where(row == r, qf[:, c0:c0 + DH], qh)
            st["q"].append(qh.astype(bf16))
        st["m"] = [jnp.full((8, DH), -jnp.inf, f32) for _ in range(hkv)]

    def step_gate_proj():
        st["g"] = jnp.dot(st["xn8"], wgbuf[...].reshape(d_model, d_ff), preferred_element_type=f32)

    def step_up_proj():
        u = jnp.dot(st["xn8"], wubuf[...].reshape(d_model, d_ff), preferred_element_type=f32)
        hid = (jax.nn.silu(st["g"]) * u).astype(bf16)
        st["hid"] = hid
        st["y"] = jnp.zeros((8, d_model), f32)
        st["hcol"] = {}
        for b in range(n_mxu_dblk, n_dblk):
            hrow = hid[0:1, b * DH:(b + 1) * DH].astype(f32) * st["gate"]
            st["hcol"][b] = jnp.transpose(jnp.broadcast_to(hrow, (DH, DH)))

    def step_k(j0):
        def run():
            for h in range(hkv):
                s = lax.dot_general(st["q"][h], kbuf[h, j0:j0 + KV_BLOCK, :],
                                    (((1,), (1,)), ((), ())),
                                    preferred_element_type=f32) * (DH ** -0.5)
                s_buf[h, :, j0:j0 + KV_BLOCK] = s
                m = st["m"][h]
                for c in range(KV_BLOCK // DH):
                    m = jnp.maximum(m, s[:, c * DH:(c + 1) * DH])
                st["m"][h] = m
            if j0 + KV_BLOCK == win:
                st["mx"] = [jnp.max(m, axis=-1, keepdims=True) for m in st["m"]]
                st["l"] = [jnp.zeros((8, DH), f32) for _ in range(hkv)]
                st["o"] = [jnp.zeros((8, DH), f32) for _ in range(hkv)]
        return run

    def step_v(j0):
        def run():
            for h in range(hkv):
                p = jnp.exp(s_buf[h, :, j0:j0 + KV_BLOCK] - st["mx"][h])
                l = st["l"][h]
                for c in range(KV_BLOCK // DH):
                    l = l + p[:, c * DH:(c + 1) * DH]
                st["l"][h] = l
                st["o"][h] = st["o"][h] + jnp.dot(p.astype(bf16), vbuf[h, j0:j0 + KV_BLOCK, :],
                                                  preferred_element_type=f32)
            if j0 + KV_BLOCK == win:
                st["on"] = [st["o"][h] / jnp.sum(st["l"][h], axis=-1, keepdims=True)
                            for h in range(hkv)]
        return run

    def step_o(r):
        def run():
            acc = st["acc"]
            for h in range(hkv):
                ob = jnp.where(row == r, st["on"][h], 0.0).astype(bf16)
                acc = acc + jnp.dot(ob, wobuf[h, r * DH:(r + 1) * DH, :],
                                    preferred_element_type=f32)
            st["acc"] = acc
        return run

    def step_down(b0, b1):
        def run():
            y = st["y"] + jnp.dot(st["hid"][:, b0 * DH:b1 * DH],
                                  wdbuf[b0:b1].reshape((b1 - b0) * DH, d_model),
                                  preferred_element_type=f32)
            st["y"] = y
            if b1 == n_mxu_dblk:
                st["acc"] = st["acc"] + jnp.where(row_d == 0, y * st["gate"], 0.0)
        return run

    def step_tail(b, r0):
        def run():
            w = wdbuf[b, r0:r0 + TAIL_ROWS, :].astype(f32)
            hc = st["hcol"][b][r0:r0 + TAIL_ROWS, :]
            hc = jnp.concatenate([hc] * (d_model // DH), axis=1)
            t = (w * hc).reshape(TAIL_ROWS // 8, 8, d_model)
            st["acc"] = st["acc"] + jnp.sum(t, axis=0)
        return run

    groups = [([(x_hbm, xbuf), (wr_hbm, wrbuf)], [xbuf, wrbuf], step_x)]
    band = d_model // NSTREAM
    for r in range(0, band, 8):
        groups.append((band_copies(wq_hbm, wqbuf, 0, NSTREAM, r, r + 8, 8, 1024),
                       [wqbuf.at[:, pl.ds(r, 8), :]], step_q if r + 8 == band else None))
    for hbm, buf, step in ((wg_hbm, wgbuf, step_gate_proj), (wu_hbm, wubuf, step_up_proj)):
        for r in range(0, band, 16):
            groups.append((band_copies(hbm, buf, 0, NSTREAM, r, r + 16, 8, d_ff // 2),
                           [buf.at[:, pl.ds(r, 16), :]], step if r + 16 == band else None))
    for hbm, buf, step in ((k_hbm, kbuf, step_k), (v_hbm, vbuf, step_v)):
        for j0 in range(0, win, KV_BLOCK):
            groups.append((kv_copies(hbm, buf, j0), [buf.at[:, pl.ds(j0, KV_BLOCK), :]], step(j0)))
    for r in range(0, rep * DH, 64):
        groups.append((band_copies(wo_hbm, wobuf, 0, hkv, r, r + 64, 16, d_model),
                       [wobuf.at[:, pl.ds(r, 64), :]],
                       step_o(r // DH) if (r + 64) % DH == 0 else None))
    for b0 in range(0, n_mxu_dblk, 4):
        groups.append((band_copies(wd_hbm, wdbuf, b0, b0 + 4, 0, DH, 16, d_model),
                       [wdbuf.at[pl.ds(b0, 4)]], step_down(b0, b0 + 4)))
    n_main = len(groups)
    for b in range(n_mxu_dblk, n_dblk):
        for r0 in range(0, DH, TAIL_ROWS):
            sl = (b, pl.ds(r0, TAIL_ROWS), slice(None))
            groups.append(([(wd_hbm.at[sl], wdbuf.at[sl])], [wdbuf.at[sl]], step_tail(b, r0)))

    seq, last_pos = [], []
    for gi, (copies, _, _) in enumerate(groups):
        for src, dst in copies:
            pos = len(seq)
            prio = 1 if (pos < LOW_START or gi >= n_main) else pos % 2
            seq.append((gi, src, dst, prio))
        last_pos.append(len(seq) - 1)

    def body(sems):
        issued = [0]

        def issue_until(end):
            while issued[0] < min(len(seq), end):
                gi, src, dst, prio = seq[issued[0]]
                pltpu.make_async_copy(src, dst, sems.at[gi]).start(priority=prio)
                issued[0] += 1

        issue_until(LOOKAHEAD)
        for gi, (_, regions, step) in enumerate(groups):
            issue_until(last_pos[gi] + 1)
            for reg in regions:
                pltpu.make_async_copy(reg, reg, sems.at[gi]).wait()
            issue_until(last_pos[gi] + 1 + LOOKAHEAD)
            if step is not None:
                step()
        o_ref[0] = jnp.sum(st["acc"], axis=0, keepdims=True).astype(o_ref.dtype)

    pl.run_scoped(body, pltpu.SemaphoreType.DMA((len(groups),)))


@jax.jit
def pallas_parallel_sum__sliding_block_cached__moe_arch_mod__decode_kernel(
    A_x: jax.Array,
    A_k_cache: jax.Array,
    A_v_cache: jax.Array,
    A_wq: jax.Array,
    A_wo: jax.Array,
    B_x: jax.Array,
    B_w_r: jax.Array,
    B_w_gate: jax.Array,
    B_w_up: jax.Array,
    B_w_down: jax.Array,
):
    del B_x
    bsz, sq, d_model = A_x.shape
    assert bsz == 1 and sq == 1
    hkv, sk = A_k_cache.shape[1], A_k_cache.shape[2]
    win = min(4096, max(256, sk // 4))
    d_ff = B_w_gate.shape[1]
    dt = A_x.dtype
    band = d_model // NSTREAM

    wq = A_wq.reshape(NSTREAM, band, HQ * DH)
    wo = A_wo.reshape(hkv, (HQ // hkv) * DH, d_model)
    wg = B_w_gate.reshape(NSTREAM, band, d_ff)
    wu = B_w_up.reshape(NSTREAM, band, d_ff)
    wd = B_w_down.reshape(d_ff // DH, DH, d_model)

    return pl.pallas_call(
        _kernel,
        out_shape=jax.ShapeDtypeStruct(A_x.shape, dt),
        in_specs=[pl.BlockSpec(memory_space=pl.ANY)] * 9,
        out_specs=pl.BlockSpec(memory_space=pltpu.VMEM),
        scratch_shapes=[
            pltpu.VMEM(A_x.shape, dt),
            pltpu.VMEM(B_w_r.shape, dt),
            pltpu.VMEM((hkv, win, DH), dt),
            pltpu.VMEM((hkv, win, DH), dt),
            pltpu.VMEM(wq.shape, dt),
            pltpu.VMEM(wo.shape, dt),
            pltpu.VMEM(wg.shape, dt),
            pltpu.VMEM(wu.shape, dt),
            pltpu.VMEM(wd.shape, dt),
            pltpu.VMEM((hkv, 8, win), jnp.float32),
        ],
        compiler_params=pltpu.CompilerParams(vmem_limit_bytes=64 * 1024 * 1024),
    )(A_x, B_w_r, A_k_cache, A_v_cache, wq, wo, wg, wu, wd)
```

```python
import jax
import jax.numpy as jnp
from jax import lax
import jax.experimental.pallas as pl
import jax.experimental.pallas.tpu as pltpu

HQ = 32
DH = 128
LN_EPS = 1e-5

NBAND = 8
KV_BLOCK = 256
KV_ROWS = 64
LOOKAHEAD = 96
LOW_START = 32
FF_STREAMS = 7
TILES_PER_COPY = 16
DOWN_ROWS = 32
DOWN_GROUPS = ((0, 3, 7, 10, 5), (1, 4, 8, 11, 2))
DOWN_TAIL = (6, 9, 12, 13)


def _interleave8(copies):
    out = []
    for i in range(0, len(copies), 8):
        c = copies[i:i + 8]
        out += [c[0], c[1], c[4], c[5], c[2], c[3], c[6], c[7]]
    return out


def _kernel(x_hbm, wr_hbm, k_hbm, v_hbm, wq_hbm, wo_hbm, wg_hbm, wu_hbm, wd_hbm, o_ref,
            xbuf, wrbuf, kbuf, vbuf, wqbuf, wobuf, wgbuf, wubuf, wdbuf, s_buf):
    f32, bf16 = jnp.float32, jnp.bfloat16
    d_model = xbuf.shape[-1]
    hkv, win, _ = kbuf.shape
    sk = k_hbm.shape[2]
    rep = HQ // hkv
    n_fblk = wdbuf.shape[0]

    st = {}
    row = lax.broadcasted_iota(jnp.int32, (8, DH), 0)
    row_d = lax.broadcasted_iota(jnp.int32, (8, d_model), 0)

    def step_x():
        x = xbuf[0].astype(f32)
        xc = x - jnp.mean(x, axis=-1, keepdims=True)
        var = jnp.mean(xc * xc, axis=-1, keepdims=True)
        xn = (xc / jnp.sqrt(var + LN_EPS)).astype(bf16).astype(f32)
        st["xn8"] = jnp.broadcast_to(xn, (8, d_model)).astype(bf16)
        r = jnp.sum(xn * wrbuf[...].astype(f32).reshape(1, d_model), axis=-1, keepdims=True)
        st["gate"] = jax.nn.sigmoid(r)
        st["acc"] = jnp.where(row_d == 0, jnp.broadcast_to(x + xn, (8, d_model)), 0.0)

    def ff_proj(buf):
        w = buf[...].reshape(d_model // 8, n_fblk, 8, DH)
        cols = [jnp.dot(st["xn8"], w[:, c].reshape(d_model, DH), preferred_element_type=f32)
                for c in range(n_fblk)]
        return jnp.concatenate(cols, axis=1)

    def step_gate_proj():
        st["g"] = ff_proj(wgbuf)

    def step_up_proj():
        hid = (jax.nn.silu(st["g"]) * ff_proj(wubuf)).astype(bf16)
        st["hid"] = hid
        st["y"] = jnp.zeros((8, d_model), f32)
        st["hcol"] = {}
        for b in DOWN_TAIL:
            hrow = hid[0:1, b * DH:(b + 1) * DH].astype(f32) * st["gate"]
            st["hcol"][b] = jnp.transpose(jnp.broadcast_to(hrow, (DH, DH)))

    def step_down(blocks):
        def run():
            y = st["y"]
            for b in blocks:
                y = y + jnp.dot(st["hid"][:, b * DH:(b + 1) * DH], wdbuf[b],
                                preferred_element_type=f32)
            st["y"] = y
            if blocks == DOWN_GROUPS[-1]:
                st["acc"] = st["acc"] + jnp.where(row_d == 0, y * st["gate"], 0.0)
        return run

    def step_q():
        qf = jnp.dot(st["xn8"], wqbuf[...].reshape(d_model, HQ * DH),
                     preferred_element_type=f32)
        st["q"] = []
        for h in range(hkv):
            qh = jnp.zeros((8, DH), f32)
            for r in range(rep):
                c0 = (h * rep + r) * DH
                qh = jnp.where(row == r, qf[:, c0:c0 + DH], qh)
            st["q"].append(qh.astype(bf16))
        st["m"] = [jnp.full((8, DH), -jnp.inf, f32) for _ in range(hkv)]

    def step_k(j0):
        def run():
            for h in range(hkv):
                s = lax.dot_general(st["q"][h], kbuf[h, j0:j0 + KV_BLOCK, :],
                                    (((1,), (1,)), ((), ())),
                                    preferred_element_type=f32) * (DH ** -0.5)
                s_buf[h, :, j0:j0 + KV_BLOCK] = s
                m = st["m"][h]
                for c in range(KV_BLOCK // DH):
                    m = jnp.maximum(m, s[:, c * DH:(c + 1) * DH])
                st["m"][h] = m
            if j0 + KV_BLOCK == win:
                st["mx"] = [jnp.max(m, axis=-1, keepdims=True) for m in st["m"]]
                st["l"] = [jnp.zeros((8, DH), f32) for _ in range(hkv)]
                st["o"] = [jnp.zeros((8, DH), f32) for _ in range(hkv)]
        return run

    def step_v(j0):
        def run():
            for h in range(hkv):
                p = jnp.exp(s_buf[h, :, j0:j0 + KV_BLOCK] - st["mx"][h])
                l = st["l"][h]
                for c in range(KV_BLOCK // DH):
                    l = l + p[:, c * DH:(c + 1) * DH]
                st["l"][h] = l
                st["o"][h] = st["o"][h] + jnp.dot(p.astype(bf16), vbuf[h, j0:j0 + KV_BLOCK, :],
                                                  preferred_element_type=f32)
            if j0 + KV_BLOCK == win:
                st["on"] = [st["o"][h] / jnp.sum(st["l"][h], axis=-1, keepdims=True)
                            for h in range(hkv)]
        return run

    def step_o(r):
        def run():
            acc = st["acc"]
            for h in range(hkv):
                ob = jnp.where(row == r, st["on"][h], 0.0).astype(bf16)
                acc = acc + jnp.dot(ob, wobuf[h, r * DH:(r + 1) * DH, :],
                                    preferred_element_type=f32)
            st["acc"] = acc
        return run

    def step_tail(b, r0):
        def run():
            w = wdbuf[b, r0:r0 + DOWN_ROWS, :].astype(f32)
            hc = st["hcol"][b][r0:r0 + DOWN_ROWS, :]
            hc = jnp.concatenate([hc] * (d_model // DH), axis=1)
            t = (w * hc).reshape(DOWN_ROWS // 8, 8, d_model)
            st["acc"] = st["acc"] + jnp.sum(t, axis=0)
        return run

    def same(hbm, buf, sl):
        return (hbm.at[sl], buf.at[sl])

    def band_copies(hbm, buf, r0, r1, rows, cols):
        return _interleave8([
            same(hbm, buf, (pl.ds(g, 2), pl.ds(r, rows), pl.ds(c, cols)))
            for r in range(r0, r1, rows)
            for c in range(0, hbm.shape[2], cols)
            for g in range(0, hbm.shape[0], 2)])

    def kv_copies(hbm, buf, j0):
        return _interleave8([
            (hbm.at[0, pl.ds(g, 2), pl.ds(sk - win + j, KV_ROWS), :],
             buf.at[pl.ds(g, 2), pl.ds(j, KV_ROWS), :])
            for j in range(j0, j0 + KV_BLOCK, KV_ROWS)
            for g in range(0, hkv, 2)])

    groups = [([(x_hbm, xbuf), (wr_hbm, wrbuf)], [xbuf, wrbuf], step_x)]
    for blocks in DOWN_GROUPS:
        groups.append(([same(wd_hbm, wdbuf, (b, pl.ds(r, DOWN_ROWS), slice(None)))
                        for r in range(0, DH, DOWN_ROWS) for b in blocks],
                       [wdbuf.at[b] for b in blocks], None))
    for hbm, buf, step in ((wg_hbm, wgbuf, step_gate_proj), (wu_hbm, wubuf, step_up_proj)):
        per = buf.shape[1]
        for j0 in range(0, per, 2):
            groups.append(([same(hbm, buf, (s, j)) for j in (j0, j0 + 1) for s in range(FF_STREAMS)],
                           [buf.at[:, pl.ds(j0, 2)]], step if j0 + 2 == per else None))
    band = d_model // NBAND
    for i, r in enumerate(range(0, band, 8)):
        step = step_down(DOWN_GROUPS[i]) if i < len(DOWN_GROUPS) else None
        groups.append((band_copies(wq_hbm, wqbuf, r, r + 8, 8, 1024),
                       [wqbuf.at[:, pl.ds(r, 8), :]], step_q if r + 8 == band else step))
    for hbm, buf, step in ((k_hbm, kbuf, step_k), (v_hbm, vbuf, step_v)):
        for j0 in range(0, win, KV_BLOCK):
            groups.append((kv_copies(hbm, buf, j0), [buf.at[:, pl.ds(j0, KV_BLOCK), :]], step(j0)))
    for r in range(0, rep * DH, 64):
        groups.append((band_copies(wo_hbm, wobuf, r, r + 64, 16, d_model),
                       [wobuf.at[:, pl.ds(r, 64), :]],
                       step_o(r // DH) if (r + 64) % DH == 0 else None))
    n_main = len(groups)
    for b in DOWN_TAIL:
        for r0 in range(0, DH, DOWN_ROWS):
            sl = (b, pl.ds(r0, DOWN_ROWS), slice(None))
            groups.append(([same(wd_hbm, wdbuf, sl)], [wdbuf.at[sl]], step_tail(b, r0)))

    seq, last_pos = [], []
    for gi, (copies, _, _) in enumerate(groups):
        for src, dst in copies:
            pos = len(seq)
            prio = 1 if (pos < LOW_START or gi >= n_main) else pos % 2
            seq.append((gi, src, dst, prio))
        last_pos.append(len(seq) - 1)

    def body(sems):
        issued = [0]

        def issue_until(end):
            while issued[0] < min(len(seq), end):
                gi, src, dst, prio = seq[issued[0]]
                pltpu.make_async_copy(src, dst, sems.at[gi]).start(priority=prio)
                issued[0] += 1

        issue_until(LOOKAHEAD)
        for gi, (_, regions, step) in enumerate(groups):
            issue_until(last_pos[gi] + 1)
            for reg in regions:
                pltpu.make_async_copy(reg, reg, sems.at[gi]).wait()
            issue_until(last_pos[gi] + 1 + LOOKAHEAD)
            if step is not None:
                step()
        o_ref[0] = jnp.sum(st["acc"], axis=0, keepdims=True).astype(o_ref.dtype)

    pl.run_scoped(body, pltpu.SemaphoreType.DMA((len(groups),)))


@jax.jit
def pallas_parallel_sum__sliding_block_cached__moe_arch_mod__decode_kernel(
    A_x: jax.Array,
    A_k_cache: jax.Array,
    A_v_cache: jax.Array,
    A_wq: jax.Array,
    A_wo: jax.Array,
    B_x: jax.Array,
    B_w_r: jax.Array,
    B_w_gate: jax.Array,
    B_w_up: jax.Array,
    B_w_down: jax.Array,
):
    del B_x
    bsz, sq, d_model = A_x.shape
    assert bsz == 1 and sq == 1
    hkv, sk = A_k_cache.shape[1], A_k_cache.shape[2]
    win = min(4096, max(256, sk // 4))
    d_ff = B_w_gate.shape[1]
    n_fblk = d_ff // DH
    assert sorted(sum(DOWN_GROUPS, DOWN_TAIL)) == list(range(n_fblk))
    dt = A_x.dtype

    def tile_view(w):
        t = w.reshape(d_model // 8, 8, n_fblk, DH).transpose(0, 2, 1, 3)
        return t.reshape(FF_STREAMS, -1, TILES_PER_COPY, 8, DH)

    wq = A_wq.reshape(NBAND, d_model // NBAND, HQ * DH)
    wo = A_wo.reshape(hkv, (HQ // hkv) * DH, d_model)
    wg = tile_view(B_w_gate)
    wu = tile_view(B_w_up)
    wd = B_w_down.reshape(n_fblk, DH, d_model)

    return pl.pallas_call(
        _kernel,
        out_shape=jax.ShapeDtypeStruct(A_x.shape, dt),
        in_specs=[pl.BlockSpec(memory_space=pl.ANY)] * 9,
        out_specs=pl.BlockSpec(memory_space=pltpu.VMEM),
        scratch_shapes=[
            pltpu.VMEM(A_x.shape, dt),
            pltpu.VMEM(B_w_r.shape, dt),
            pltpu.VMEM((hkv, win, DH), dt),
            pltpu.VMEM((hkv, win, DH), dt),
            pltpu.VMEM(wq.shape, dt),
            pltpu.VMEM(wo.shape, dt),
            pltpu.VMEM(wg.shape, dt),
            pltpu.VMEM(wu.shape, dt),
            pltpu.VMEM(wd.shape, dt),
            pltpu.VMEM((hkv, 8, win), jnp.float32),
        ],
        compiler_params=pltpu.CompilerParams(vmem_limit_bytes=64 * 1024 * 1024),
    )(A_x, B_w_r, A_k_cache, A_v_cache, wq, wo, wg, wu, wd)
```

```python
import jax
import jax.numpy as jnp
from jax import lax
import jax.experimental.pallas as pl
import jax.experimental.pallas.tpu as pltpu

HQ = 32
DH = 128
LN_EPS = 1e-5

UNIT = 16
CUT = 14
STREAM_ORDER = (0, 2, 1, 3, 4, 6, 5, 7)
FF_STREAMS = 7
KV_BLOCK = 256
LOOKAHEAD = 96
LOW_START = 32
DOWN_ROWS = 32
DOWN_GROUPS = ((0, 3, 7, 10, 5), (1, 4, 8, 11, 2))
DOWN_TAIL = (6, 9, 12, 13)


def _kernel(x_hbm, wr_hbm, k_hbm, v_hbm, wq_hbm, wo_hbm, wg_hbm, wu_hbm, wd_hbm, o_ref,
            xbuf, wrbuf, kbuf, vbuf, wqbuf, wobuf, wgbuf, wubuf, wdbuf, s_buf):
    f32, bf16 = jnp.float32, jnp.bfloat16
    d_model = xbuf.shape[-1]
    hkv, win, _ = kbuf.shape
    sk = k_hbm.shape[2]
    rep = HQ // hkv
    n_fblk = wdbuf.shape[0]
    n_dblk = d_model // DH

    st = {}
    row = lax.broadcasted_iota(jnp.int32, (8, DH), 0)
    row_d = lax.broadcasted_iota(jnp.int32, (8, d_model), 0)

    def tile_cols(tiles, n_col):
        t = tiles.reshape(-1, n_col, 8, DH)
        return [t[:, c].reshape(-1, DH) for c in range(n_col)]

    def mm(a, b):
        return jnp.dot(a, b, preferred_element_type=f32)

    def step_x():
        x = xbuf[0].astype(f32)
        xc = x - jnp.mean(x, axis=-1, keepdims=True)
        var = jnp.mean(xc * xc, axis=-1, keepdims=True)
        xn = (xc / jnp.sqrt(var + LN_EPS)).astype(bf16).astype(f32)
        st["xn8"] = jnp.broadcast_to(xn, (8, d_model)).astype(bf16)
        r = jnp.sum(xn * wrbuf[...].astype(f32).reshape(1, d_model), axis=-1, keepdims=True)
        st["gate"] = jax.nn.sigmoid(r)
        st["acc"] = jnp.where(row_d == 0, jnp.broadcast_to(x + xn, (8, d_model)), 0.0)

    def ff_proj(buf):
        return jnp.concatenate([mm(st["xn8"], w) for w in tile_cols(buf[...], n_fblk)], axis=1)

    def step_gate_proj():
        st["g"] = ff_proj(wgbuf)

    def step_up_proj():
        hid = (jax.nn.silu(st["g"]) * ff_proj(wubuf)).astype(bf16)
        st["hid"] = hid
        st["y"] = jnp.zeros((8, d_model), f32)
        st["hcol"] = {}
        for b in DOWN_TAIL:
            hrow = hid[0:1, b * DH:(b + 1) * DH].astype(f32) * st["gate"]
            st["hcol"][b] = jnp.transpose(jnp.broadcast_to(hrow, (DH, DH)))

    def step_down(blocks):
        def run():
            y = st["y"]
            for b in blocks:
                y = y + mm(st["hid"][:, b * DH:(b + 1) * DH], wdbuf[b])
            st["y"] = y
            if blocks == DOWN_GROUPS[-1]:
                st["acc"] = st["acc"] + jnp.where(row_d == 0, y * st["gate"], 0.0)
        return run

    def step_q():
        wcols = tile_cols(wqbuf[...], HQ)
        st["q"] = []
        for h in range(hkv):
            qh = jnp.zeros((8, DH), f32)
            for r in range(rep):
                qh = jnp.where(row == r, mm(st["xn8"], wcols[h * rep + r]), qh)
            st["q"].append(qh.astype(bf16))
        st["m"] = [jnp.full((8, DH), -jnp.inf, f32) for _ in range(hkv)]

    def step_k(j0):
        def run():
            for h in range(hkv):
                s = lax.dot_general(st["q"][h], kbuf[h, j0:j0 + KV_BLOCK, :],
                                    (((1,), (1,)), ((), ())),
                                    preferred_element_type=f32) * (DH ** -0.5)
                s_buf[h, :, j0:j0 + KV_BLOCK] = s
                m = st["m"][h]
                for c in range(KV_BLOCK // DH):
                    m = jnp.maximum(m, s[:, c * DH:(c + 1) * DH])
                st["m"][h] = m
            if j0 + KV_BLOCK == win:
                st["mx"] = [jnp.max(m, axis=-1, keepdims=True) for m in st["m"]]
                st["l"] = [jnp.zeros((8, DH), f32) for _ in range(hkv)]
                st["o"] = [jnp.zeros((8, DH), f32) for _ in range(hkv)]
        return run

    def step_v(j0):
        def run():
            for h in range(hkv):
                p = jnp.exp(s_buf[h, :, j0:j0 + KV_BLOCK] - st["mx"][h])
                l = st["l"][h]
                for c in range(KV_BLOCK // DH):
                    l = l + p[:, c * DH:(c + 1) * DH]
                st["l"][h] = l
                st["o"][h] = st["o"][h] + mm(p.astype(bf16), vbuf[h, j0:j0 + KV_BLOCK, :])
            if j0 + KV_BLOCK == win:
                st["on"] = [st["o"][h] / jnp.sum(st["l"][h], axis=-1, keepdims=True)
                            for h in range(hkv)]
        return run

    def step_o(r):
        per_head = (DH // 8) * n_dblk

        def run():
            acc = st["acc"]
            for h in range(hkv):
                ob = jnp.where(row == r, st["on"][h], 0.0).astype(bf16)
                t0 = (h * rep + r) * per_head
                wcols = tile_cols(wobuf[t0:t0 + per_head], n_dblk)
                acc = acc + jnp.concatenate([mm(ob, w) for w in wcols], axis=1)
            st["acc"] = acc
        return run

    def step_tail(b, r0):
        def run():
            w = wdbuf[b, r0:r0 + DOWN_ROWS, :].astype(f32)
            hc = st["hcol"][b][r0:r0 + DOWN_ROWS, :]
            hc = jnp.concatenate([hc] * n_dblk, axis=1)
            t = (w * hc).reshape(DOWN_ROWS // 8, 8, d_model)
            st["acc"] = st["acc"] + jnp.sum(t, axis=0)
        return run

    def same(hbm, buf, *sl):
        return (hbm.at[sl], buf.at[sl])

    def band_rounds(hbm, buf):
        n_tiles = buf.shape[0]
        per = n_tiles // len(STREAM_ORDER)
        rounds = []
        for u in range(per // UNIT):
            copies = []
            for b in STREAM_ORDER:
                hi = b * per + CUT + u * UNIT
                lo = max(hi - UNIT, 0)
                copies.append(same(hbm, buf, pl.ds(lo, hi - lo)))
            rounds.append(copies)
        rounds[-1].append(same(hbm, buf, pl.ds(n_tiles - (UNIT - CUT), UNIT - CUT)))
        return rounds

    def kv_copies(hbm, buf, j0, j1):
        cuts = sorted({j0, j1} | {c for c in range(CUT * 8, j1, UNIT * 8) if c > j0})
        copies = []
        for s0, s1 in zip(cuts[:-1], cuts[1:]):
            src_rows, dst_rows = pl.ds(sk - win + s0, s1 - s0), pl.ds(s0, s1 - s0)
            if (s1 - s0) * hkv <= UNIT * 8:
                copies.append((hbm.at[0, :, src_rows, :], buf.at[:, dst_rows, :]))
            else:
                copies += [(hbm.at[0, h, src_rows, :], buf.at[h, dst_rows, :])
                           for h in STREAM_ORDER]
        return copies

    groups = [([(x_hbm, xbuf), (wr_hbm, wrbuf)], step_x)]
    for blocks in DOWN_GROUPS:
        groups.append(([same(wd_hbm, wdbuf, b, pl.ds(r, DOWN_ROWS))
                        for r in range(0, DH, DOWN_ROWS) for b in blocks], None))
    for hbm, buf, step in ((wg_hbm, wgbuf, step_gate_proj), (wu_hbm, wubuf, step_up_proj)):
        per = buf.shape[0] // FF_STREAMS
        for t0 in range(0, per, 2 * UNIT):
            groups.append(([same(hbm, buf, pl.ds(s * per + t, UNIT))
                            for t in (t0, t0 + UNIT) for s in range(FF_STREAMS)],
                           step if t0 + 2 * UNIT == per else None))
    rounds = band_rounds(wq_hbm, wqbuf)
    for i in range(len(rounds) // 2):
        step = step_down(DOWN_GROUPS[i]) if i < len(DOWN_GROUPS) else None
        groups.append((rounds[2 * i] + rounds[2 * i + 1],
                       step_q if 2 * i + 2 == len(rounds) else step))
    for hbm, buf, step in ((k_hbm, kbuf, step_k), (v_hbm, vbuf, step_v)):
        for j in range(0, win, KV_BLOCK):
            j0 = j + CUT * 8 if j else 0
            j1 = min(win, j + KV_BLOCK + CUT * 8)
            groups.append((kv_copies(hbm, buf, j0, j1), step(j)))
    rounds = band_rounds(wo_hbm, wobuf)
    for r0, r1, r in ((0, 3, None), (3, 5, 0), (5, 7, None), (7, 9, 1),
                      (9, 11, None), (11, 13, 2), (13, 15, None), (15, 16, 3)):
        groups.append((sum(rounds[r0:r1], []), None if r is None else step_o(r)))
    n_main = len(groups)
    for b in DOWN_TAIL:
        for r0 in range(0, DH, DOWN_ROWS):
            groups.append(([same(wd_hbm, wdbuf, b, pl.ds(r0, DOWN_ROWS))], step_tail(b, r0)))

    seq, last_pos = [], []
    for gi, (copies, _) in enumerate(groups):
        for src, dst in copies:
            pos = len(seq)
            prio = 1 if (pos < LOW_START or gi >= n_main) else pos % 2
            seq.append((gi, src, dst, prio))
        last_pos.append(len(seq) - 1)

    def body(sems):
        issued = [0]

        def issue_until(end):
            while issued[0] < min(len(seq), end):
                gi, src, dst, prio = seq[issued[0]]
                pltpu.make_async_copy(src, dst, sems.at[gi]).start(priority=prio)
                issued[0] += 1

        issue_until(LOOKAHEAD)
        for gi, (copies, step) in enumerate(groups):
            issue_until(last_pos[gi] + 1)
            for src, dst in copies:
                pltpu.make_async_copy(src, dst, sems.at[gi]).wait()
            issue_until(last_pos[gi] + 1 + LOOKAHEAD)
            if step is not None:
                step()
        o_ref[0] = jnp.sum(st["acc"], axis=0, keepdims=True).astype(o_ref.dtype)

    pl.run_scoped(body, pltpu.SemaphoreType.DMA((len(groups),)))


@jax.jit
def pallas_parallel_sum__sliding_block_cached__moe_arch_mod__decode_kernel(
    A_x: jax.Array,
    A_k_cache: jax.Array,
    A_v_cache: jax.Array,
    A_wq: jax.Array,
    A_wo: jax.Array,
    B_x: jax.Array,
    B_w_r: jax.Array,
    B_w_gate: jax.Array,
    B_w_up: jax.Array,
    B_w_down: jax.Array,
):
    del B_x
    bsz, sq, d_model = A_x.shape
    assert bsz == 1 and sq == 1 and d_model == 512
    hkv, sk = A_k_cache.shape[1], A_k_cache.shape[2]
    assert hkv == len(STREAM_ORDER)
    win = min(4096, max(256, sk // 4))
    n_fblk = B_w_gate.shape[1] // DH
    assert sorted(sum(DOWN_GROUPS, DOWN_TAIL)) == list(range(n_fblk))
    dt = A_x.dtype

    def tile_view(w):
        r, c = w.shape
        return w.reshape(r // 8, 8, c // DH, DH).transpose(0, 2, 1, 3).reshape(-1, 8, DH)

    wq, wo, wg, wu = (tile_view(w) for w in (A_wq, A_wo, B_w_gate, B_w_up))
    wd = B_w_down.reshape(n_fblk, DH, d_model)

    return pl.pallas_call(
        _kernel,
        out_shape=jax.ShapeDtypeStruct(A_x.shape, dt),
        in_specs=[pl.BlockSpec(memory_space=pl.ANY)] * 9,
        out_specs=pl.BlockSpec(memory_space=pltpu.VMEM),
        scratch_shapes=[
            pltpu.VMEM(A_x.shape, dt),
            pltpu.VMEM(B_w_r.shape, dt),
            pltpu.VMEM((hkv, win, DH), dt),
            pltpu.VMEM((hkv, win, DH), dt),
            pltpu.VMEM(wq.shape, dt),
            pltpu.VMEM(wo.shape, dt),
            pltpu.VMEM(wg.shape, dt),
            pltpu.VMEM(wu.shape, dt),
            pltpu.VMEM(wd.shape, dt),
            pltpu.VMEM((hkv, 8, win), jnp.float32),
        ],
        compiler_params=pltpu.CompilerParams(vmem_limit_bytes=64 * 1024 * 1024),
    )(A_x, B_w_r, A_k_cache, A_v_cache, wq, wo, wg, wu, wd)
```

```python
import jax
import jax.numpy as jnp
from jax import lax
import jax.experimental.pallas as pl
import jax.experimental.pallas.tpu as pltpu

HQ = 32
DH = 128
LN_EPS = 1e-5

UNIT = 16
CUT = 14
STREAM_ORDER = (0, 2, 1, 3, 4, 6, 5, 7)
KV_BLOCK = 256
LOOKAHEAD = 96
LOW_START = 32
DOWN_ROWS = 32
DOWN_GROUPS = ((0, 3, 6, 9, 2, 5), (10, 11, 12, 13))
DOWN_TAIL = (1, 4, 7, 8)


def _kernel(x_hbm, wr_hbm, k_hbm, v_hbm, wq_hbm, wo_hbm, wg_hbm, wu_hbm, wd_hbm, o_ref,
            xbuf, wrbuf, kbuf, vbuf, wqbuf, wobuf, wgbuf, wubuf, wdbuf, s_buf):
    f32, bf16 = jnp.float32, jnp.bfloat16
    d_model = xbuf.shape[-1]
    hkv, win, _ = kbuf.shape
    sk = k_hbm.shape[2]
    rep = HQ // hkv
    n_fblk = wdbuf.shape[0]
    n_dblk = d_model // DH

    st = {}
    row = lax.broadcasted_iota(jnp.int32, (8, DH), 0)
    row_d = lax.broadcasted_iota(jnp.int32, (8, d_model), 0)

    def tile_cols(tiles, n_col):
        t = tiles.reshape(-1, n_col, 8, DH)
        return [t[:, c].reshape(-1, DH) for c in range(n_col)]

    def mm(a, b):
        return jnp.dot(a, b, preferred_element_type=f32)

    def step_x():
        x = xbuf[0].astype(f32)
        xc = x - jnp.mean(x, axis=-1, keepdims=True)
        var = jnp.mean(xc * xc, axis=-1, keepdims=True)
        xn = (xc / jnp.sqrt(var + LN_EPS)).astype(bf16).astype(f32)
        st["xn8"] = jnp.broadcast_to(xn, (8, d_model)).astype(bf16)
        r = jnp.sum(xn * wrbuf[...].astype(f32).reshape(1, d_model), axis=-1, keepdims=True)
        st["gate"] = jax.nn.sigmoid(r)
        st["acc"] = jnp.where(row_d == 0, jnp.broadcast_to(x + xn, (8, d_model)), 0.0)

    def ff_proj(buf):
        return jnp.concatenate([mm(st["xn8"], w) for w in tile_cols(buf[...], n_fblk)], axis=1)

    def step_gate_proj():
        st["g"] = ff_proj(wgbuf)

    def step_up_proj():
        hid = (jax.nn.silu(st["g"]) * ff_proj(wubuf)).astype(bf16)
        st["hid"] = hid
        st["y"] = jnp.zeros((8, d_model), f32)
        st["hcol"] = {}
        for b in DOWN_TAIL:
            hrow = hid[0:1, b * DH:(b + 1) * DH].astype(f32) * st["gate"]
            st["hcol"][b] = jnp.transpose(jnp.broadcast_to(hrow, (DH, DH)))

    def step_down(blocks):
        def run():
            y = st["y"]
            for b in blocks:
                y = y + mm(st["hid"][:, b * DH:(b + 1) * DH], wdbuf[b])
            st["y"] = y
            if blocks == DOWN_GROUPS[-1]:
                st["acc"] = st["acc"] + jnp.where(row_d == 0, y * st["gate"], 0.0)
        return run

    def step_q():
        wcols = tile_cols(wqbuf[...], HQ)
        st["q"] = []
        for h in range(hkv):
            qh = jnp.zeros((8, DH), f32)
            for r in range(rep):
                qh = jnp.where(row == r, mm(st["xn8"], wcols[h * rep + r]), qh)
            st["q"].append(qh.astype(bf16))
        st["m"] = [jnp.full((8, DH), -jnp.inf, f32) for _ in range(hkv)]

    def step_k(j0):
        def run():
            for h in range(hkv):
                s = lax.dot_general(st["q"][h], kbuf[h, j0:j0 + KV_BLOCK, :],
                                    (((1,), (1,)), ((), ())),
                                    preferred_element_type=f32) * (DH ** -0.5)
                s_buf[h, :, j0:j0 + KV_BLOCK] = s
                m = st["m"][h]
                for c in range(KV_BLOCK // DH):
                    m = jnp.maximum(m, s[:, c * DH:(c + 1) * DH])
                st["m"][h] = m
            if j0 + KV_BLOCK == win:
                st["mx"] = [jnp.max(m, axis=-1, keepdims=True) for m in st["m"]]
                st["l"] = [jnp.zeros((8, DH), f32) for _ in range(hkv)]
                st["o"] = [jnp.zeros((8, DH), f32) for _ in range(hkv)]
        return run

    def step_v(j0):
        def run():
            for h in range(hkv):
                p = jnp.exp(s_buf[h, :, j0:j0 + KV_BLOCK] - st["mx"][h])
                l = st["l"][h]
                for c in range(KV_BLOCK // DH):
                    l = l + p[:, c * DH:(c + 1) * DH]
                st["l"][h] = l
                st["o"][h] = st["o"][h] + mm(p.astype(bf16), vbuf[h, j0:j0 + KV_BLOCK, :])
            if j0 + KV_BLOCK == win:
                st["on"] = [st["o"][h] / jnp.sum(st["l"][h], axis=-1, keepdims=True)
                            for h in range(hkv)]
        return run

    def step_o(r):
        per_head = (DH // 8) * n_dblk

        def run():
            acc = st["acc"]
            for h in range(hkv):
                ob = jnp.where(row == r, st["on"][h], 0.0).astype(bf16)
                t0 = (h * rep + r) * per_head
                wcols = tile_cols(wobuf[t0:t0 + per_head], n_dblk)
                acc = acc + jnp.concatenate([mm(ob, w) for w in wcols], axis=1)
            st["acc"] = acc
        return run

    def step_tail(b, r0):
        def run():
            w = wdbuf[b, r0:r0 + DOWN_ROWS, :].astype(f32)
            hc = st["hcol"][b][r0:r0 + DOWN_ROWS, :]
            hc = jnp.concatenate([hc] * n_dblk, axis=1)
            t = (w * hc).reshape(DOWN_ROWS // 8, 8, d_model)
            st["acc"] = st["acc"] + jnp.sum(t, axis=0)
        return run

    def same(hbm, buf, *sl):
        return (hbm.at[sl], buf.at[sl])

    def band_rounds(hbm, buf):
        n_tiles = buf.shape[0]
        per = n_tiles // len(STREAM_ORDER)
        rounds = []
        for u in range(per // UNIT):
            copies = []
            for b in STREAM_ORDER:
                hi = b * per + CUT + u * UNIT
                lo = max(hi - UNIT, 0)
                copies.append(same(hbm, buf, pl.ds(lo, hi - lo)))
            rounds.append(copies)
        rounds[-1].append(same(hbm, buf, pl.ds(n_tiles - (UNIT - CUT), UNIT - CUT)))
        return rounds

    def kv_copies(hbm, buf, j0, j1):
        cuts = sorted({j0, j1} | {c for c in range(CUT * 8, j1, UNIT * 8) if c > j0})
        copies = []
        for s0, s1 in zip(cuts[:-1], cuts[1:]):
            src_rows, dst_rows = pl.ds(sk - win + s0, s1 - s0), pl.ds(s0, s1 - s0)
            if (s1 - s0) * hkv <= UNIT * 8:
                copies.append((hbm.at[0, :, src_rows, :], buf.at[:, dst_rows, :]))
            else:
                copies += [(hbm.at[0, h, src_rows, :], buf.at[h, dst_rows, :])
                           for h in STREAM_ORDER]
        return copies

    groups = [([(x_hbm, xbuf), (wr_hbm, wrbuf)], step_x)]
    groups.append(([same(wd_hbm, wdbuf, b, pl.ds(r, DOWN_ROWS))
                    for r in range(0, DH, DOWN_ROWS) for b in DOWN_GROUPS[0]], None))
    units = ([same(wd_hbm, wdbuf, b, pl.ds(r, DOWN_ROWS))
              for b in DOWN_GROUPS[1] for r in range(0, DH, DOWN_ROWS)]
             + [same(wu_hbm, wubuf, pl.ds(t, UNIT)) for t in range(0, wubuf.shape[0], UNIT)]
             + [same(wg_hbm, wgbuf, pl.ds(t, UNIT)) for t in range(0, wgbuf.shape[0], UNIT)])
    per = len(units) // len(STREAM_ORDER)
    assert per * len(STREAM_ORDER) == len(units) and per % 2 == 0
    for j0 in range(0, per, 2):
        groups.append(([units[k * per + j] for j in (j0, j0 + 1) for k in STREAM_ORDER],
                       step_gate_proj if j0 + 2 == per else None))
    rounds = band_rounds(wq_hbm, wqbuf)
    steps = [step_up_proj] + [step_down(blocks) for blocks in DOWN_GROUPS]
    steps += [None] * (len(rounds) // 2 - 1 - len(steps)) + [step_q]
    for i, step in enumerate(steps):
        groups.append((rounds[2 * i] + rounds[2 * i + 1], step))
    for hbm, buf, step in ((k_hbm, kbuf, step_k), (v_hbm, vbuf, step_v)):
        for j in range(0, win, KV_BLOCK):
            j0 = j + CUT * 8 if j else 0
            j1 = min(win, j + KV_BLOCK + CUT * 8)
            groups.append((kv_copies(hbm, buf, j0, j1), step(j)))
    rounds = band_rounds(wo_hbm, wobuf)
    for r0, r1, r in ((0, 3, None), (3, 5, 0), (5, 7, None), (7, 9, 1),
                      (9, 11, None), (11, 13, 2), (13, 15, None), (15, 16, 3)):
        groups.append((sum(rounds[r0:r1], []), None if r is None else step_o(r)))
    n_main = len(groups)
    for b in DOWN_TAIL:
        for r0 in range(0, DH, DOWN_ROWS):
            groups.append(([same(wd_hbm, wdbuf, b, pl.ds(r0, DOWN_ROWS))], step_tail(b, r0)))

    seq, last_pos = [], []
    for gi, (copies, _) in enumerate(groups):
        for src, dst in copies:
            pos = len(seq)
            prio = 1 if (pos < LOW_START or gi >= n_main) else pos % 2
            seq.append((gi, src, dst, prio))
        last_pos.append(len(seq) - 1)

    def body(sems):
        issued = [0]

        def issue_until(end):
            while issued[0] < min(len(seq), end):
                gi, src, dst, prio = seq[issued[0]]
                pltpu.make_async_copy(src, dst, sems.at[gi]).start(priority=prio)
                issued[0] += 1

        issue_until(LOOKAHEAD)
        for gi, (copies, step) in enumerate(groups):
            issue_until(last_pos[gi] + 1)
            for src, dst in copies:
                pltpu.make_async_copy(src, dst, sems.at[gi]).wait()
            issue_until(last_pos[gi] + 1 + LOOKAHEAD)
            if step is not None:
                step()
        o_ref[0] = jnp.sum(st["acc"], axis=0, keepdims=True).astype(o_ref.dtype)

    pl.run_scoped(body, pltpu.SemaphoreType.DMA((len(groups),)))


@jax.jit
def pallas_parallel_sum__sliding_block_cached__moe_arch_mod__decode_kernel(
    A_x: jax.Array,
    A_k_cache: jax.Array,
    A_v_cache: jax.Array,
    A_wq: jax.Array,
    A_wo: jax.Array,
    B_x: jax.Array,
    B_w_r: jax.Array,
    B_w_gate: jax.Array,
    B_w_up: jax.Array,
    B_w_down: jax.Array,
):
    del B_x
    bsz, sq, d_model = A_x.shape
    assert bsz == 1 and sq == 1 and d_model == 512
    hkv, sk = A_k_cache.shape[1], A_k_cache.shape[2]
    assert hkv == len(STREAM_ORDER)
    win = min(4096, max(256, sk // 4))
    n_fblk = B_w_gate.shape[1] // DH
    assert sorted(sum(DOWN_GROUPS, DOWN_TAIL)) == list(range(n_fblk))
    dt = A_x.dtype

    def tile_view(w):
        r, c = w.shape
        return w.reshape(r // 8, 8, c // DH, DH).transpose(0, 2, 1, 3).reshape(-1, 8, DH)

    wq, wo, wg, wu = (tile_view(w) for w in (A_wq, A_wo, B_w_gate, B_w_up))
    wd = B_w_down.reshape(n_fblk, DH, d_model)

    return pl.pallas_call(
        _kernel,
        out_shape=jax.ShapeDtypeStruct(A_x.shape, dt),
        in_specs=[pl.BlockSpec(memory_space=pl.ANY)] * 9,
        out_specs=pl.BlockSpec(memory_space=pltpu.VMEM),
        scratch_shapes=[
            pltpu.VMEM(A_x.shape, dt),
            pltpu.VMEM(B_w_r.shape, dt),
            pltpu.VMEM((hkv, win, DH), dt),
            pltpu.VMEM((hkv, win, DH), dt),
            pltpu.VMEM(wq.shape, dt),
            pltpu.VMEM(wo.shape, dt),
            pltpu.VMEM(wg.shape, dt),
            pltpu.VMEM(wu.shape, dt),
            pltpu.VMEM(wd.shape, dt),
            pltpu.VMEM((hkv, 8, win), jnp.float32),
        ],
        compiler_params=pltpu.CompilerParams(vmem_limit_bytes=64 * 1024 * 1024),
    )(A_x, B_w_r, A_k_cache, A_v_cache, wq, wo, wg, wu, wd)
```
